```python
import os as _os
_os.environ.setdefault("JAX_PLATFORMS", "cpu")
import jax
import jax.numpy as jnp

def _softmax(x, axis=-1):
    return jax.nn.softmax(x, axis=axis)
def _gelu(x):
    return jax.nn.gelu(x, approximate=True)
def _silu(x):
    return jax.nn.silu(x)
def _sigmoid(x):
    return jax.nn.sigmoid(x)
def _layernorm(x, axis=-1, eps=1e-5):
    m = jnp.mean(x, axis=axis, keepdims=True)
    v = jnp.var(x, axis=axis, keepdims=True)
    return (x - m) / jnp.sqrt(v + eps)
def _scatter_add(tgt, idx, src, axis=0):
    return tgt.at[idx].add(src)
def _segment_sum(src, seg, n):
    return jax.ops.segment_sum(src, seg, n)
class _Rng:
    def __init__(self, key):
        self._k = key
    def _next(self):
        self._k, sub = jax.random.split(self._k)
        return sub
    def normal(self, shape):
        return jax.random.normal(self._next(), shape, dtype=jnp.bfloat16)
    def randint(self, lo, hi, shape):
        return jax.random.randint(self._next(), shape, lo, hi, dtype=jnp.int32)
    def uniform(self, shape, lo=0.0, hi=1.0):
        return jax.random.uniform(self._next(), shape, jnp.bfloat16, lo, hi)
    def permutation(self, n):
        return jax.random.permutation(self._next(), n)


kernel_name = 'gated_mix__linear_attn_block__swiglu_ffn__prompt'

def setup_inputs():
    _rng = _Rng(jax.random.key(int.from_bytes(__import__("os").urandom(4), "little")))
    _w = (lambda a: (lambda t: t.astype(jnp.bfloat16) if jnp.issubdtype(t.dtype, jnp.floating) else t)(jnp.asarray(a)))
    def _A_setup():
        B, S, D = 1, 2048, 512
        return {
            "x": _w((lambda *s: _rng.normal(s) * 0.05)(B, S, D)),
            "wqkv": _w((lambda *s: _rng.normal(s) * 0.8)(D, 3 * D)),
            "wo": _w((lambda *s: _rng.normal(s) * 0.05)(D, D)),
        }
    _A_in = _A_setup()

    def _B_setup():
        B, S, D, F = 1, 2048, 512, 1792
        return {
            "x": _w((lambda *s: _rng.normal(s) * 0.05)(B, S, D)),
            "w_gate": _w((lambda *s: _rng.normal(s) * 0.1)(D, F)),
            "w_up": _w((lambda *s: _rng.normal(s) * 0.1)(D, F)),
            "w_down": _w((lambda *s: _rng.normal(s) * 0.1)(F, D)),
        }
    _B_in = _B_setup()

    return {
        "A_x": _A_in["x"],
        "A_wqkv": _A_in["wqkv"],
        "A_wo": _A_in["wo"],
        "B_x": _B_in["x"],
        "B_w_gate": _B_in["w_gate"],
        "B_w_up": _B_in["w_up"],
        "B_w_down": _B_in["w_down"],
        "gate_w": _w((lambda *s: _rng.normal(s) * 0.05)(512) * 16.0),
    }

def reference(A_x, A_wqkv, A_wo, B_x, B_w_gate, B_w_up, B_w_down, gate_w):
    def _A_ref(x, wqkv, wo):
        B, S, D = x.shape
        H = 32; Dh = D // H
        qkv = (lambda x, *d: x.transpose(*d))((x @ wqkv).reshape(B, S, 3, H, Dh), 2, 0, 3, 1, 4)
        q, k, v = qkv[0], qkv[1], qkv[2]
        phi = lambda t: jnp.where(t > 0, t + 1, jnp.exp(t)) + 1e-6
        pq, pk = phi(q), phi(k)
        kv = jnp.einsum("bhsd,bhse->bhde", pk, v)
        z = jnp.einsum("bhsd->bhd", pk)
        num = jnp.einsum("bhqd,bhde->bhqe", pq, kv)
        den = jnp.einsum("bhqd,bhd->bhq", pq, z)[..., None] + 1e-6
        o = num / den
        return (lambda x, *d: x.transpose(*d))(o, 0, 2, 1, 3).reshape(B, S, D) @ wo

    def _B_ref(x, w_gate, w_up, w_down):
        g = _silu(x @ w_gate)
        u = x @ w_up
        return (g * u) @ w_down

    x = A_x
    g = _sigmoid((x * gate_w).sum(-1, keepdims=True))
    a = _A_ref(x, A_wqkv, A_wo)
    b = _B_ref(x, B_w_gate, B_w_up, B_w_down)
    return g * a + (1 - g) * b
```

```python
import functools
import jax, jax.numpy as jnp
from jax import lax
import jax.experimental.pallas as pl
import jax.experimental.pallas.tpu as pltpu

S, D, F, H = 2048, 512, 1792, 32
DH = D // H
Q = S // 4
T = 128
f32, bf16 = jnp.float32, jnp.bfloat16

def _add(a, b): return a + b
def _sub(a, b): return a - b
def _ladd(a, b): return [p + q for p, q in zip(a, b)]
def _lsub(a, b): return [p - q for p, q in zip(a, b)]

def lhs1(a11, a12, a21, a22, add, sub):
    return [lambda: add(a11, a22), lambda: add(a21, a22), lambda: a11, lambda: a22,
            lambda: add(a11, a12), lambda: sub(a21, a11), lambda: sub(a12, a22)]
def rhs1(b11, b12, b21, b22, add, sub):
    return [lambda: add(b11, b22), lambda: b11, lambda: sub(b12, b22), lambda: sub(b21, b11),
            lambda: b22, lambda: add(b11, b12), lambda: add(b21, b22)]
RHS_AS_LHS = (0, 2, 6, 5, 3, 4, 1)

def operands(side, blk):
    quad = lambda I, J: [blk(2 * I + i, 2 * J + j) for i in range(2) for j in range(2)]
    outer = side(quad(0, 0), quad(0, 1), quad(1, 0), quad(1, 1), _ladd, _lsub)
    cache = {}
    def get(R, r):
        if R not in cache:
            cache[R] = side(*outer[R](), _add, _sub)
        return cache[R][r]()
    return get

def c_seq(prod, add, sub, emit):
    m1 = prod(0); m2 = prod(1); m3 = prod(2)
    emit(1, 1, add(sub(add(prod(5), m1), m2), m3))
    m4 = prod(3)
    emit(1, 0, add(m4, m2)); t = add(m4, m1)
    m5 = prod(4)
    emit(0, 1, add(m5, m3)); t = sub(t, m5)
    emit(0, 0, add(prod(6), t))

def c_quad(prod, add, sub, emit):
    m1 = prod(0); m4 = prod(3); m5 = prod(4); m7 = prod(6)
    emit(0, 0, add(add(sub(m7, m5), m1), m4))
    m2 = prod(1); m3 = prod(2); m6 = prod(5)
    emit(1, 0, add(m2, m4)); emit(0, 1, add(m3, m5)); emit(1, 1, add(add(sub(m6, m2), m3), m1))

def strassen2(prod, emit, inner, extra=None, done=None):
    def outer(R):
        o = [None] * 4
        def em(i, j, v): o[2 * i + j] = v
        inner(lambda r: prod(R, r), _add, _sub, em)
        if extra is not None:
            o = _ladd(extra(R), o)
        return o
    def oem(I, J, vals):
        for i in range(2):
            for j in range(2):
                emit(2 * I + i, 2 * J + j, vals[2 * i + j])
        if done is not None: done(I, J)
    c_seq(outer, _ladd, _lsub, oem)

def mm(a, b): return jnp.dot(a, b, preferred_element_type=f32)
def mm_nt(a, b): return lax.dot_general(a, b, (((1,), (1,)), ((), ())), preferred_element_type=f32)
def phi(t): return jnp.where(t > 0, t + 1.0, jnp.exp(t)) + 1e-6
def tile(i): return slice(i * T, (i + 1) * T)

def make(chunks=(64, 192, 256), opaque="smem", flags=None, ohb=True):
    assert sum(chunks) == Q
    nc = len(chunks)
    offs = [sum(chunks[:c]) for c in range(nc)]
    def kernel(x_hbm, wqkv_hbm, wo_hbm, wg_hbm, wu_hbm, wd_hbm, gw_hbm, o_hbm,
               x_v, wqkv_v, wo_v, wg_v, wu_v, wd_v, gw_v, o_v, xa, wa, h, g1, g0, pkt, zc, gm, mm_v, zs, sems, osems):
        nsem = [0]
        def copy(src, dst):
            c = pltpu.make_async_copy(src, dst, sems.at[nsem[0]]); nsem[0] += 1
            return c
        def cols(hbm, v, lo, hi): return copy(hbm.at[:, lo:hi], v.at[:, lo:hi])
        c_x = [copy(x_hbm.at[:, pl.ds(offs[c], chunks[c])], x_v.at[:, pl.ds(offs[c], chunks[c])]) for c in range(nc)]
        c_u0 = cols(wu_hbm, wu_v, 0, 512)
        c_gw = copy(gw_hbm, gw_v)
        c_k = cols(wqkv_hbm, wqkv_v, D, 2 * D)
        c_g0 = cols(wg_hbm, wg_v, 0, 512)
        c_rest = [cols(wu_hbm, wu_v, 512, F), cols(wg_hbm, wg_v, 512, F), cols(wqkv_hbm, wqkv_v, 2 * D, 3 * D),
                  copy(wo_hbm, wo_v), cols(wqkv_hbm, wqkv_v, 0, D), copy(wd_hbm, wd_v)]
        for c in [c_u0, c_x[0], c_gw] + c_x[1:] + [c_k, c_g0] + c_rest: c.start()

        if opaque == "smem":
            def zinit(i, _):
                zs[i] = 0
                return 0
            lax.fori_loop(0, 16, zinit, 0)
            nz = [0]
            def fresh():
                nz[0] += 1
                return zs[nz[0] - 1]
        else:
            fresh = lambda: 0

        def wblocks(ref, c0, scale=None):
            def blk(i, j):
                v = ref[tile(i), c0 + j * T:c0 + (j + 1) * T].astype(f32)
                return v if scale is None else v * scale
            return blk

        c_u0.wait()
        w = operands(rhs1, wblocks(wu_v, 0))
        for R in range(7):
            for r in range(7):
                wa[7 * R + r] = w(R, r).astype(bf16)
        for c in range(nc):
            c_x[c].wait()
            if c == 0:
                c_gw.wait()
                gw = gw_v[...].astype(f32).reshape(1, D)
            rows = pl.ds(offs[c], chunks[c])
            for r0 in range(offs[c], offs[c] + chunks[c], 16):
                xb = [[x_v[i, pl.ds(r0, 16), tile(j)].astype(f32) for j in range(4)] for i in range(4)]
                a = operands(lhs1, lambda i, j: xb[i][j])
                for R in range(7):
                    for r in range(7):
                        xa[7 * R + r, pl.ds(r0, 16), :] = a(R, r).astype(bf16)
                for i in range(4):
                    t = sum(xb[i][j] * gw[:, tile(j)] for j in range(1, 4)) + xb[i][0] * gw[:, tile(0)]
                    th = 0.5 * jnp.tanh(0.5 * jnp.sum(t, axis=1, keepdims=True))
                    g1[i, pl.ds(r0, 16), :] = jnp.broadcast_to(0.5 + th, (16, T))
                    g0[i, pl.ds(r0, 16), :] = jnp.broadcast_to(0.5 - th, (16, T))
            z = fresh()
            def emit(i, j, v): h[j, i, rows, :] = v
            strassen2(lambda R, r: mm(xa[7 * R + r + z, rows, :], wa[7 * R + r + z]), emit, c_quad)

        def up(s):
            z = fresh()
            w = operands(rhs1, wblocks(wu_v, 512 * s))
            def emit(i, j, v): h[4 * s + j, i] = v * g0[i + z]
            strassen2(lambda R, r: mm(xa[7 * R + r + z], w(R, r).astype(bf16)), emit, c_quad)
        def gate(s):
            z = fresh()
            w = operands(rhs1, wblocks(wg_v, 512 * s, 0.5))
            def emit(i, j, v):
                u = h[4 * s + j + z, i]
                if s == 0: u = u * g0[i + z]
                h[4 * s + j + z, i] = (v * jnp.tanh(v) + v) * u
            strassen2(lambda R, r: mm(xa[7 * R + r + z], w(R, r).astype(bf16)), emit, c_quad)
        def transposed(c0, emit):
            z = fresh()
            blk = wblocks(wqkv_v, c0)
            w = operands(rhs1, lambda i, j: blk(i, j).T)
            strassen2(lambda R, r: mm_nt(w(R, r).astype(bf16), xa[7 * R + r + z]), emit, c_seq)

        c_k.wait()
        zsum = {}
        def emit_k(i, j, v):
            p = phi(v)
            pkt[j, i] = p
            t = (p[:, tile(0)] + p[:, tile(1)]) + (p[:, tile(2)] + p[:, tile(3)])
            zsum[j] = t + zsum[j] if j in zsum else t
        transposed(D, emit_k)
        for j in range(4):
            zc[j] = jnp.broadcast_to(jnp.sum(zsum[j], axis=1, keepdims=True), (T, T))
        c_g0.wait()
        gate(0)
        z = fresh()
        a = operands(lhs1, lambda i, j: pkt[i + z, j])
        def emit_g(i, j, v): gm[i, :, tile(j)] = v.astype(bf16)
        strassen2(lambda R, r: mm(a(R, r).astype(bf16), xa[7 * RHS_AS_LHS[R] + RHS_AS_LHS[r] + z]), emit_g, c_seq)
        for c in c_rest: c.wait()
        up(1)
        same_head = (lax.broadcasted_iota(jnp.int32, (T, T), 0) // DH) == (lax.broadcasted_iota(jnp.int32, (T, T), 1) // DH)
        kv = [jnp.where(same_head, mm(gm[j], wqkv_v[:, 2 * D + j * T:2 * D + (j + 1) * T]), 0.0).astype(bf16) for j in range(4)]
        gate(1)
        for j in range(4):
            mm_v[j] = mm(kv[j], wo_v[tile(j), :])
        zq = fresh()
        def emit_q(i, j, v):
            p = phi(v)
            outs = []
            for t in range(4):
                pt = p[:, tile(t)].reshape(T // DH, DH, T)
                den = jnp.sum(pt * zc[j + zq].reshape(T // DH, DH, T), axis=1, keepdims=True) + 1e-6
                o = (pt * pltpu.reciprocal(den, approx=False)).reshape(T, T).T
                h[14 + j, i, tile(t), :] = o * g1[i + zq, tile(t), :]
        transposed(0, emit_q)
        up(2); gate(2)
        z = fresh()
        lo = lax.broadcasted_iota(jnp.int32, (T, T), 1) < 64
        wl = {}
        for i in range(4):
            for e in range(2):
                gg = wg_v[tile(i), tile(12 + e)].astype(f32) * 0.5
                uu = wu_v[tile(i), tile(12 + e)].astype(f32)
                rr = pltpu.roll(jnp.where(lo, uu, gg), 64, 1)
                wl[i, 2 * e] = jnp.where(lo, gg, rr)
                wl[i, 2 * e + 1] = jnp.where(lo, rr, uu)
        w = operands(rhs1, lambda i, j: wl[i, j])
        loq = lax.broadcasted_iota(jnp.int32, (Q, T), 1) < 64
        pend = {}
        def emit_l(i, j, v):
            pend[i, j] = v
            if j % 2 == 1:
                c0, c1 = pend[i, j - 1], v
                rr = pltpu.roll(jnp.where(loq, c1, c0), 64, 1)
                gg, uu = jnp.where(loq, c0, rr), jnp.where(loq, rr, c1)
                h[12 + j // 2, i] = (gg * jnp.tanh(gg) + gg) * (uu * g0[i + z])
        strassen2(lambda R, r: mm(xa[7 * R + r + z], w(R, r).astype(bf16)), emit_l, c_quad)

        z = fresh() if ohb else 0
        base = (0, 4, 8, 14)
        aa = [operands(lhs1, lambda i, j, b=b: h[b + j + z, i]) for b in base]
        bb = [operands(rhs1, lambda i, j, s=s: wd_v[tile(4 * s + i), tile(j)].astype(f32)) for s in range(3)]
        bb.append(operands(rhs1, lambda i, j: mm_v[i + z, :, tile(j)]))
        hq = lambda I, J: [h[12 + J + z, 2 * I + i] for i in range(2)]
        wq = lambda I, J: [wd_v[tile(12 + I), tile(2 * J + j)].astype(f32) for j in range(2)]
        al = lhs1(hq(0, 0), hq(0, 1), hq(1, 0), hq(1, 1), _ladd, _lsub)
        bl = rhs1(wq(0, 0), wq(0, 1), wq(1, 0), wq(1, 1), _ladd, _lsub)
        def extra(R):
            av, bv = [v.astype(bf16) for v in al[R]()], [v.astype(bf16) for v in bl[R]()]
            return [mm(av[i], bv[j]) for i in range(2) for j in range(2)]
        def prod(R, r):
            return mm(jnp.concatenate([a(R, r).astype(bf16) for a in aa], axis=1),
                      jnp.concatenate([b(R, r).astype(bf16) for b in bb], axis=0))
        def emit_o(i, j, v): o_v[i, :, tile(j)] = v.astype(bf16)
        ocs = []
        def done(I, J):
            sl = (slice(2 * I, 2 * I + 2), slice(None), slice(256 * J, 256 * J + 256))
            c = pltpu.make_async_copy(o_v.at[sl], o_hbm.at[sl], osems.at[len(ocs)])
            c.start(); ocs.append(c)
        strassen2(prod, emit_o, c_seq, extra, done)
        for c in ocs: c.wait()

    def fn(A_x, A_wqkv, A_wo, B_x, B_w_gate, B_w_up, B_w_down, gate_w):
        anyspec = pl.BlockSpec(memory_space=pl.ANY)
        out = pl.pallas_call(
            kernel,
            in_specs=[anyspec] * 7,
            out_specs=anyspec,
            out_shape=jax.ShapeDtypeStruct((4, Q, D), bf16),
            scratch_shapes=[
                pltpu.VMEM((4, Q, D), bf16), pltpu.VMEM((D, 3 * D), bf16), pltpu.VMEM((D, D), bf16),
                pltpu.VMEM((D, F), bf16), pltpu.VMEM((D, F), bf16), pltpu.VMEM((F, D), bf16), pltpu.VMEM((D,), bf16),
                pltpu.VMEM((4, Q, D), bf16),
                pltpu.VMEM((49, Q, T), bf16), pltpu.VMEM((49, T, T), bf16), pltpu.VMEM((18, 4, Q, T), f32),
                pltpu.VMEM((4, Q, T), f32), pltpu.VMEM((4, Q, T), f32), pltpu.VMEM((4, 4, T, Q), f32),
                pltpu.VMEM((4, T, T), f32), pltpu.VMEM((4, T, D), bf16), pltpu.VMEM((4, T, D), f32),
                pltpu.SMEM((16,), jnp.int32),
                pltpu.SemaphoreType.DMA((nc + 10,)), pltpu.SemaphoreType.DMA((4,)),
            ],
            compiler_params=pltpu.CompilerParams(vmem_limit_bytes=120 * 1024 * 1024, flags=flags),
        )(A_x.reshape(4, Q, D), A_wqkv, A_wo, B_w_gate, B_w_up, B_w_down, gate_w)
        return out.reshape(1, S, D)
    return fn


_impl = make()


@jax.jit
def pallas_gated_mix__linear_attn_block__swiglu_ffn__prompt_kernel(
    A_x, A_wqkv, A_wo, B_x, B_w_gate, B_w_up, B_w_down, gate_w):
    return _impl(A_x, A_wqkv, A_wo, B_x, B_w_gate, B_w_up, B_w_down, gate_w)
```

```python
import functools

import jax
import jax.numpy as jnp
from jax import lax
import jax.experimental.pallas as pl
import jax.experimental.pallas.tpu as pltpu

S, D, F, H = 2048, 512, 1792, 32
DH = D // H
T = 128
Q = S // 4
GROUPS = F // D
REST = F - GROUPS * D
PAD = DH + 1
PAD_ROWS = H * (PAD + 1)

WK_SLABS = 4
X_CHUNKS = (32, 32, 32, 64, 96)
X_PART = sum(X_CHUNKS)
X_ROWS = 32
SIDE_ROWS = 64
SIDE_LAG = 8
N_ZEROS = 128

W1_GATE, W1_UP, W1_Q, W1_REST, W1_SIZE = 0, 8, 12, 16, 20
W2_V, W2_O, W2_GATE, W2_UP, W2_DOWN = 0, 4, 8, 12, 16
W2_SIZE = W2_DOWN + F // T

f32, bf16, i32 = jnp.float32, jnp.bfloat16, jnp.int32


def _add(a, b):
    return [p + q for p, q in zip(a, b)]


def _sub(a, b):
    return [p - q for p, q in zip(a, b)]


def _lhs_sum(n, a):
    return (
        lambda: _add(a(0, 0), a(1, 1)),
        lambda: _add(a(1, 0), a(1, 1)),
        lambda: a(0, 0),
        lambda: a(1, 1),
        lambda: _add(a(0, 0), a(0, 1)),
        lambda: _sub(a(1, 0), a(0, 0)),
        lambda: _sub(a(0, 1), a(1, 1)),
    )[n]()


RHS_AS_LHS = (0, 2, 6, 5, 3, 4, 1)


def _rhs_sum(n, b):
    return _lhs_sum(RHS_AS_LHS[n], b)


def _operands(side, load):
    outer = {}

    def get(R, r):
        if R not in outer:
            outer[R] = side(R, lambda I, J: [
                load(2 * I + i, 2 * J + j, R) for i in range(2) for j in range(2)])
        return side(r, lambda i, j: [outer[R][2 * i + j]])[0]

    return get


def _combine_spread(prod, emit, park=lambda n, v: lambda: v):
    m2, m4 = prod(1), prod(3)
    emit(1, 0, _add(m4, m2))
    m3, m5 = prod(2), prod(4)
    emit(0, 1, _add(m5, m3))
    m1 = prod(0)
    t1, t2 = park(0, _sub(_add(m1, m4), m5)), park(1, _sub(_add(m1, m3), m2))
    emit(0, 0, _add(prod(6), t1()))
    emit(1, 1, _add(prod(5), t2()))


def _combine_lazy(prod, emit):
    m2, m4 = prod(1), prod(3)
    emit(1, 0, _add(m4, m2))
    m3, m5 = prod(2), prod(4)
    emit(0, 1, _add(m5, m3))
    t = _sub(m4, m5)
    m1 = prod(0)
    emit(0, 0, _add(_add(prod(6), m1), t))
    emit(1, 1, _sub(_add(_add(prod(5), m1), m3), m2))


def _combine_4_3(prod, emit):
    m2, m4, m3, m5 = prod(1), prod(3), prod(2), prod(4)
    emit(1, 0, _add(m4, m2))
    emit(0, 1, _add(m5, m3))
    t1, t2 = _sub(m4, m5), _sub(m3, m2)
    m1, m7, m6 = prod(0), prod(6), prod(5)
    emit(0, 0, _add(_add(m7, m1), t1))
    emit(1, 1, _add(_add(m6, m1), t2))


def _combine_3_4(prod, emit):
    m2, m4, m1 = prod(1), prod(3), prod(0)
    emit(1, 0, _add(m4, m2))
    t1, t2 = _add(m1, m4), _sub(m1, m2)
    m3, m5, m7, m6 = prod(2), prod(4), prod(6), prod(5)
    emit(0, 1, _add(m5, m3))
    emit(0, 0, _add(_sub(m7, m5), t1))
    emit(1, 1, _add(_add(m6, m3), t2))


def _combine_chain(prod, emit):
    m3, m5 = prod(2), prod(4)
    emit(0, 1, _add(m5, m3))
    t = _sub(prod(6), m5)
    m4, m2 = prod(3), prod(1)
    emit(1, 0, _add(m2, m4))
    u = _sub(m3, m2)
    m1 = prod(0)
    emit(0, 0, _add(_add(m1, t), m4))
    emit(1, 1, _add(_add(prod(5), m1), u))


_COMBINE_BY_MXU = (_combine_4_3, _combine_3_4, _combine_spread, _combine_spread)


def _strassen2(prod, emit, inner, outer, extra=None):
    done = []

    def outer_prod(R):
        add = extra(R) if extra and done else None
        out = [None] * 4

        def put(i, j, v):
            out[2 * i + j] = v[0] + add[2 * i + j] if add else v[0]

        inner()(lambda r: [prod(R, r)], put)
        done.append(R)
        return _add(extra(R), out) if extra and not add else out

    def outer_emit(I, J, tiles):
        for i, j in ((0, 1), (1, 0), (0, 0), (1, 1)):
            emit(2 * I + i, 2 * J + j, tiles[2 * i + j])

    outer(outer_prod, outer_emit)


def _dot(a, b, dims=((1,), (0,))):
    return lax.dot_general(a, b, (dims, ((), ())), preferred_element_type=f32)


def _phi(t):
    return jnp.where(t > 0, t + 1.0, jnp.exp(t)) + 1e-6


def _silu_of_twice(t):
    return t * jnp.tanh(t) + t


def _tile(i):
    return slice(i * T, (i + 1) * T)


def _repeat(v, rows):
    return jnp.concatenate([v] * (rows // 8), axis=0)


def _fold(v):
    acc = v[:8]
    for r in range(8, v.shape[0], 8):
        acc = acc + v[r:r + 8]
    return acc


def _swap_halves(a, b):
    low = lax.broadcasted_iota(i32, a.shape, 1) < T // 2
    moved = pltpu.roll(jnp.where(low, b, a), T // 2, 1)
    return jnp.where(low, a, moved), jnp.where(low, moved, b)


def _store_heads(ref, n, j, v):
    for h in range(T // DH):
        ref[n, pl.ds((j * (T // DH) + h) * PAD, DH), :] = v[h * DH:(h + 1) * DH]


def _load_d_major(ref, n, j):
    return jnp.concatenate(
        [ref[n, pl.ds(4 * j + d, H, stride=PAD), :] for d in range(4)], axis=0)


def _kernel(x_hbm, wqkv_hbm, wo_hbm, wg_hbm, wu_hbm, wd_hbm, gw_hbm, o_hbm,
            x, wk, wu0, w1, w2, gw, out,
            x_sums, wk_sums, pk, hidden, pq, rest, ffn_gate, q_scale,
            z, z_rows, gram, m_rows, wq_rows, w_rest, parked,
            zeros, first_sems, sems):
    copy = pltpu.make_async_copy
    slab = T // WK_SLABS
    parts = Q // X_PART

    def copy_wk(c):
        rows = pl.ds(pl.multiple_of(c * slab, slab), slab)
        return copy(wqkv_hbm.at[:, rows, pl.ds(D, D)], wk.at[:, rows], first_sems.at[c])

    def copy_x(part, c):
        start = part * X_PART + sum(X_CHUNKS[:c])
        rows = pl.ds(pl.multiple_of(start, 16), X_CHUNKS[c])
        sem = first_sems.at[WK_SLABS + part * len(X_CHUNKS) + c]
        return copy(x_hbm.at[:, rows], x.at[:, rows], sem)

    for c in range(WK_SLABS):
        copy_wk(c).start()
    for part in range(parts):
        for c in range(len(X_CHUNKS)):
            copy_x(part, c).start()

    @pl.loop(0, N_ZEROS // 8)
    def _(n):
        for e in range(8):
            zeros[n * 8 + e] = 0

    used = []

    def zero():
        used.append(None)
        return zeros[len(used) - 1]

    def zero_per_product():
        return functools.lru_cache(None)(lambda R: zero())

    issued = [0]

    def by_mxu():
        issued[0] += 7
        return _COMBINE_BY_MXU[(issued[0] - 7) % 4]

    def with_side_jobs(lhs, rhs, dot, jobs):
        tie = zero()
        start = {n * (49 - SIDE_LAG) // len(jobs): job for n, job in enumerate(jobs)}
        due, count = {}, [0]

        def prod(R, r):
            n, b = count[0], rhs(R, r)
            if due.get(n) is not None:
                nothing = pltpu.bitcast(pltpu.bitcast(due[n], i32) & tie, f32)
                b = jnp.concatenate([b[:8] + nothing, b[8:]], axis=0)
            v = dot(lhs(R, r, tie), b.astype(bf16))
            if n in start:
                row = (n % 4) * (v.shape[0] // 8)
                due[n + SIDE_LAG] = start[n](pltpu.bitcast(v[row:row + 8], i32) & tie)
            count[0] += 1
            return v

        return prod, tie

    def project(load, emit, jobs=(), dot=_dot, busy=True):
        prod, tie = with_side_jobs(
            lambda R, r, tie: x_sums[7 * R + r + tie], _operands(_rhs_sum, load), dot, jobs)

        def park(n, tiles):
            for e, v in enumerate(tiles):
                parked[4 * n + e][0] = v
            return lambda: [parked[4 * n + e][tie] for e in range(4)]

        outer = functools.partial(_combine_spread, park=park) if busy else _combine_spread
        _strassen2(prod, lambda i, j, v: emit(i, j, v, tie), by_mxu, outer)

    def tiles_of(ref, n, scale=None):
        off = zero_per_product()

        def load(i, j, R):
            v = ref[n + i + off(R), :, _tile(j)].astype(f32)
            return v if scale is None else v * scale

        return load

    @pl.loop(0, WK_SLABS)
    def _(c):
        copy_wk(c).wait()
        for r0 in range(0, slab, 16):
            rows = pl.ds(pl.multiple_of(c * slab + r0, 16), 16)
            packed_rows = pl.ds(pl.multiple_of(c * (slab // 2) + r0 // 2, 8), 8)
            w = [[wk[i, rows, _tile(j)].astype(f32) for j in range(4)] for i in range(4)]
            sums = _operands(_rhs_sum, lambda i, j, R: w[i][j])
            for n in range(49):
                wk_sums[n, packed_rows, :] = pltpu.bitcast(sums(n // 7, n % 7).astype(bf16), i32)

    def columns(hbm, start, buf, n, sem):
        return copy(hbm.at[:, :, pl.ds(start, D)], buf.at[pl.ds(n, 4)], sem)

    copy_gw, copy_wu0 = copy(gw_hbm, gw, sems.at[0]), columns(wu_hbm, 0, wu0, 0, sems.at[1])
    sem1, sem2, out_sem = sems.at[2], sems.at[3], sems.at[4]
    copy_gw.start()
    copy_wu0.start()
    for c in (
        columns(wg_hbm, 0, w1, W1_GATE, sem1),
        columns(wu_hbm, D, w1, W1_UP, sem1),
        columns(wg_hbm, D, w1, W1_GATE + 4, sem1),
        columns(wqkv_hbm, 0, w1, W1_Q, sem1),
        copy(wg_hbm.at[:, :, pl.ds(GROUPS * D, REST)],
             w1.at[pl.ds(W1_REST, 4), :, pl.ds(0, REST)], sem1),
        copy(wu_hbm.at[:, :, pl.ds(GROUPS * D, REST)],
             w1.at[pl.ds(W1_REST, 4), :, pl.ds(REST, REST)], sem1),
        columns(wg_hbm, 2 * D, w2, W2_GATE, sem2),
        columns(wu_hbm, 2 * D, w2, W2_UP, sem2),
        columns(wqkv_hbm, 2 * D, w2, W2_V, sem2),
        copy(wo_hbm, w2.at[pl.ds(W2_O, 4)], sem2),
        copy(wd_hbm, w2.at[pl.ds(W2_DOWN, F // T)], sem2),
    ):
        c.start(priority=1)

    @pl.loop(0, parts)
    def _(part):
        off = zero_per_product()
        for c, size in enumerate(X_CHUNKS):
            copy_x(part, c).wait()
            for r0 in range(sum(X_CHUNKS[:c]), sum(X_CHUNKS[:c]) + size, X_ROWS):
                rows = pl.ds(pl.multiple_of(part * X_PART + r0, 16), X_ROWS)
                sums = _operands(
                    _lhs_sum, lambda i, j, R: x[i + off(R), rows, _tile(j)].astype(f32))
                tie = zero()

                def prod(R, r):
                    a = sums(R, r)
                    x_sums[pl.ds(7 * R + r, 1), rows, :] = a[None].astype(bf16)
                    return _dot(a.astype(bf16), pltpu.bitcast(wk_sums[7 * R + r + tie], bf16))

                def emit(i, j, v):
                    pk[j, i, rows] = _phi(v)

                _strassen2(prod, emit, by_mxu, _combine_spread)

    copy_gw.wait()
    copy_wu0.wait()

    half_gw = jnp.broadcast_to(gw[...].astype(f32).reshape(1, D) * 0.5, (8, D))

    def mix_gate(i, rows, nothing):
        nothing = pltpu.bitcast(nothing, f32)
        t = [x[i, rows, _tile(j)].astype(f32) * _repeat(half_gw[:, _tile(j)] + nothing, SIDE_ROWS)
             for j in range(4)]
        t = jnp.sum((t[0] + t[1]) + (t[2] + t[3]), axis=1, keepdims=True)
        t = jnp.broadcast_to(0.5 * jnp.tanh(t), (SIDE_ROWS, T))
        ffn_gate[i, rows] = 0.5 - t
        return _fold(t)

    def z_to_rows(j, nothing):
        total = jnp.sum(z[j] + pltpu.bitcast(nothing, f32), axis=0, keepdims=True)
        _store_heads(z_rows, 0, j, jnp.broadcast_to(total, (T, T)).T)

    def z_from_rows(j, nothing):
        v = _load_d_major(z_rows, 0, j) + _repeat(pltpu.bitcast(nothing, f32), T)
        z[4 + j] = v.T[:8]

    def wq_to_rows(i, j, nothing):
        w = pltpu.bitcast(w1[W1_Q + i, :, _tile(j)], i32) | _repeat(nothing, T // 2)
        _store_heads(wq_rows, i, j, pltpu.bitcast(w, bf16).T.astype(f32))

    def pair_rest(i, j, nothing):
        half = _repeat(0.5 + pltpu.bitcast(nothing, f32), T)
        a, b = _swap_halves(w1[W1_REST + i, :, _tile(j)].astype(f32) * half,
                            w1[W1_REST + i, :, _tile(2 + j)].astype(f32))
        w_rest[2 * j, _tile(i)] = a.astype(bf16)
        w_rest[2 * j + 1, _tile(i)] = b.astype(bf16)

    norm_off = zero_per_product()

    def normalise(i, rows, nothing):
        nothing, off = pltpu.bitcast(nothing, f32), norm_off(0)
        t = [pq[j + off, i, rows] * _repeat(z[4 + j + off] + nothing, SIDE_ROWS) for j in range(4)]
        den = (t[0] + t[1]) + (t[2] + t[3])
        den = den + pltpu.roll(den, 2 * H, 1)
        den = den + pltpu.roll(den, H, 1)
        q_scale[i, rows] = (1.0 - ffn_gate[i + off, rows]) * pltpu.reciprocal(den + 1e-6, full_range=False)

    def over_rows(job, quarters):
        return [functools.partial(job, i, pl.ds(r0, SIDE_ROWS))
                for i in quarters for r0 in range(0, Q, SIDE_ROWS)]

    def over_tiles(job, n):
        return [functools.partial(job, i, j) for i in range(4) for j in range(n)]

    off = zero_per_product()
    pk_sums = _operands(_lhs_sum, lambda i, j, R: pk[i + off(R), j])

    def pk_operand(R, r):
        v = pk_sums(R, r)
        if R in (1, 4) and r in (1, 4):
            z[2 * (R == 1) + (r == 1)] = _fold(v)
        return v

    def emit_gram(i, j, v):
        gram[i, _tile(j)] = v.astype(bf16)

    prod, _ = with_side_jobs(
        lambda R, r, tie: x_sums[7 * RHS_AS_LHS[R] + RHS_AS_LHS[r] + tie], pk_operand,
        functools.partial(_dot, dims=((0,), (0,))), over_rows(mix_gate, range(4)))
    _strassen2(prod, emit_gram, lambda: _combine_chain, _combine_chain)
    issued[0] = 0

    def up(s, ref, n, jobs=()):
        def emit(i, j, v, tie):
            hidden[s][j, i] = v * ffn_gate[i + tie]

        project(tiles_of(ref, n), emit, jobs, busy=False)

    def gate(s, ref, n, jobs=()):
        def emit(i, j, v, tie):
            u = hidden[s][j + tie, i]
            hidden[s][j + tie, i] = _silu_of_twice(v) * u

        project(tiles_of(ref, n, 0.5), emit, jobs)

    up(0, wu0, 0, [functools.partial(job, j) for job in (z_to_rows, z_from_rows) for j in range(4)])
    copy(w1, w1, sem1).wait()
    gate(0, w1, W1_GATE, over_tiles(pair_rest, 2))
    up(1, w1, W1_UP, over_tiles(wq_to_rows, 4))
    gate(1, w1, W1_GATE + 4)
    pl.delay(1)
    copy(w2, w2, sem2).wait()

    tie = zero()
    same_head = (lax.broadcasted_iota(i32, (T, T), 0) // DH
                 == lax.broadcasted_iota(i32, (T, T), 1) // DH)
    kv = []
    for j in range(4):
        wv = jnp.concatenate([w2[W2_V + i, :, _tile(j)] for i in range(4)], axis=0)
        g = pltpu.bitcast(pltpu.bitcast(gram[j + tie].T, i32) | tie, bf16)
        kv.append(jnp.where(same_head, _dot(g, wv), 0.0).astype(bf16))
    for j in range(4):
        m = _dot(kv[j], w2[W2_O + j])
        for n in range(4):
            _store_heads(m_rows, n, j, m[:, _tile(n)])

    def emit_q(i, j, v, tie):
        pq[j, i] = _phi(v)

    q_off = zero_per_product()
    project(lambda i, j, R: _load_d_major(wq_rows, i + q_off(R), j), emit_q,
            dot=functools.partial(_dot, dims=((1,), (1,))))
    up(2, w2, W2_UP, over_rows(normalise, (2, 3, 0, 1)))
    gate(2, w2, W2_GATE)

    waiting = {}

    def emit_rest(i, j, v, tie):
        waiting[i, j] = v
        if (i, j ^ 1) in waiting:
            g, u = _swap_halves(waiting[i, j & 2], waiting[i, j | 1])
            rest[j // 2, i] = _silu_of_twice(g) * (u * ffn_gate[i + tie])

    rest_off = zero_per_product()
    project(lambda i, j, R: w_rest[j + rest_off(R), _tile(i)].astype(f32), emit_rest)

    o = zero_per_product()
    lhs = [_operands(_lhs_sum, lambda i, j, R, s=s: hidden[s][j + o(R), i]) for s in range(GROUPS)]
    lhs.append(_operands(_lhs_sum, lambda i, j, R: pq[j + o(R), i] * q_scale[i + o(R)]))
    rhs = [_operands(_rhs_sum,
                     lambda i, j, R, s=s: w2[W2_DOWN + 4 * s + i + o(R), :, _tile(j)].astype(f32))
           for s in range(GROUPS)]
    rhs.append(_operands(_rhs_sum, lambda i, j, R: _load_d_major(m_rows, j + o(R), i)))

    def prod_out(R, r):
        return _dot(jnp.concatenate([a(R, r) for a in lhs], axis=1).astype(bf16),
                    jnp.concatenate([b(R, r) for b in rhs], axis=0).astype(bf16))

    def prod_rest(R):
        a = _lhs_sum(R, lambda I, J: [rest[J + o(R), 2 * I + i] for i in range(2)])
        b = _rhs_sum(R, lambda I, J: [
            w2[W2_DOWN + 4 * GROUPS + I + o(R), :, _tile(2 * J + j)].astype(f32) for j in range(2)])
        return [_dot(a[i].astype(bf16), b[j].astype(bf16)) for i in range(2) for j in range(2)]

    written = []

    def emit_out(i, j, v):
        written.append(None)
        cuts = (0, Q) if len(written) < 16 else (0, Q // 2, 3 * Q // 4, Q)
        for lo, hi in zip(cuts, cuts[1:]):
            out[j, i, lo:hi] = v[lo:hi].astype(bf16)
            copy(out.at[j, i, lo:hi], o_hbm.at[i, lo:hi, _tile(j)], out_sem).start()

    _strassen2(prod_out, emit_out, lambda: _combine_chain, _combine_lazy, prod_rest)
    copy(o_hbm, o_hbm, out_sem).wait()


@jax.jit
def pallas_gated_mix__linear_attn_block__swiglu_ffn__prompt_kernel(
    A_x: jax.Array,
    A_wqkv: jax.Array,
    A_wo: jax.Array,
    B_x: jax.Array,
    B_w_gate: jax.Array,
    B_w_up: jax.Array,
    B_w_down: jax.Array,
    gate_w: jax.Array,
):
    del B_x
    vmem = pltpu.VMEM
    tiles = vmem((4, 4, Q, T), f32)
    out = pl.pallas_call(
        _kernel,
        in_specs=[pl.BlockSpec(memory_space=pl.ANY)] * 7,
        out_specs=pl.BlockSpec(memory_space=pl.ANY),
        out_shape=jax.ShapeDtypeStruct((4, Q, D), bf16),
        scratch_shapes=[
            vmem((4, Q, D), bf16),
            vmem((4, T, D), bf16),
            vmem((4, T, D), bf16),
            vmem((W1_SIZE, T, D), bf16),
            vmem((W2_SIZE, T, D), bf16),
            vmem((D,), bf16),
            vmem((4, 4, Q, T), bf16),
            vmem((49, Q, T), bf16),
            vmem((49, T // 2, T), i32),
            tiles,
            [tiles] * GROUPS,
            tiles,
            vmem((2, 4, Q, T), f32),
            vmem((4, Q, T), f32),
            vmem((4, Q, T), f32),
            vmem((8, 8, T), f32),
            vmem((1, PAD_ROWS, T), f32),
            vmem((4, D, T), bf16),
            vmem((4, PAD_ROWS, T), f32),
            vmem((4, PAD_ROWS, T), f32),
            vmem((4, D, T), bf16),
            [vmem((2, Q, T), f32)] * 8,
            pltpu.SMEM((N_ZEROS,), i32),
            pltpu.SemaphoreType.DMA((WK_SLABS + Q // X_PART * len(X_CHUNKS),)),
            pltpu.SemaphoreType.DMA((5,)),
        ],
        compiler_params=pltpu.CompilerParams(
            vmem_limit_bytes=100 * 1024 * 1024,
            disable_semaphore_checks=True,
            flags={"XLA_TPU_RESCHEDULE_DMA_DONES": True},
        ),
    )(
        A_x.reshape(4, Q, D),
        A_wqkv.reshape(4, T, 3 * D),
        A_wo.reshape(4, T, D),
        B_w_gate.reshape(4, T, F),
        B_w_up.reshape(4, T, F),
        B_w_down.reshape(F // T, T, D),
        gate_w,
    )
    return out.reshape(1, S, D)
```

```python
import functools

import jax
import jax.numpy as jnp
from jax import lax
import jax.experimental.pallas as pl
import jax.experimental.pallas.tpu as pltpu

S, D, F, H = 2048, 512, 1792, 32
DH = D // H
T = 128
Q = S // 4
GROUPS = F // D
REST = F - GROUPS * D
PAD = DH + 1
PAD_ROWS = H * (PAD + 1)

WK_ROWS = 16
X_ROWS = 32
X_UNROLL = 8
SIDE_ROWS = 64
SIDE_LAG = 8
N_ZEROS = 128

W1_GATE, W1_UP, W1_Q, W1_REST, W1_SIZE = 0, 8, 12, 16, 20
W2_V, W2_O, W2_GATE, W2_UP, W2_DOWN = 0, 4, 8, 12, 16
W2_SIZE = W2_DOWN + F // T

f32, bf16, i32 = jnp.float32, jnp.bfloat16, jnp.int32


def _add(a, b):
    return [p + q for p, q in zip(a, b)]


def _sub(a, b):
    return [p - q for p, q in zip(a, b)]


def _lhs_sum(n, a):
    return (
        lambda: _add(a(0, 0), a(1, 1)),
        lambda: _add(a(1, 0), a(1, 1)),
        lambda: a(0, 0),
        lambda: a(1, 1),
        lambda: _add(a(0, 0), a(0, 1)),
        lambda: _sub(a(1, 0), a(0, 0)),
        lambda: _sub(a(0, 1), a(1, 1)),
    )[n]()


RHS_AS_LHS = (0, 2, 6, 5, 3, 4, 1)


def _rhs_sum(n, b):
    return _lhs_sum(RHS_AS_LHS[n], b)


def _operands(side, load):
    outer = {}

    def get(R, r):
        if R not in outer:
            outer[R] = side(R, lambda I, J: [
                load(2 * I + i, 2 * J + j, R) for i in range(2) for j in range(2)])
        return side(r, lambda i, j: [outer[R][2 * i + j]])[0]

    return get


def _combine_spread(prod, emit, park=lambda n, v: lambda: v):
    m2, m4 = prod(1), prod(3)
    emit(1, 0, _add(m4, m2))
    m3, m5 = prod(2), prod(4)
    emit(0, 1, _add(m5, m3))
    m1 = prod(0)
    t1, t2 = park(0, _sub(_add(m1, m4), m5)), park(1, _sub(_add(m1, m3), m2))
    emit(0, 0, _add(prod(6), t1()))
    emit(1, 1, _add(prod(5), t2()))


def _combine_4_3(prod, emit):
    m2, m4, m3, m5 = prod(1), prod(3), prod(2), prod(4)
    emit(1, 0, _add(m4, m2))
    emit(0, 1, _add(m5, m3))
    t1, t2 = _sub(m4, m5), _sub(m3, m2)
    m1, m7, m6 = prod(0), prod(6), prod(5)
    emit(0, 0, _add(_add(m7, m1), t1))
    emit(1, 1, _add(_add(m6, m1), t2))


def _combine_3_4(prod, emit):
    m2, m4, m1 = prod(1), prod(3), prod(0)
    emit(1, 0, _add(m4, m2))
    t1, t2 = _add(m1, m4), _sub(m1, m2)
    m3, m5, m7, m6 = prod(2), prod(4), prod(6), prod(5)
    emit(0, 1, _add(m5, m3))
    emit(0, 0, _add(_sub(m7, m5), t1))
    emit(1, 1, _add(_add(m6, m3), t2))


def _combine_chain(prod, emit):
    m3, m5 = prod(2), prod(4)
    emit(0, 1, _add(m5, m3))
    t = _sub(prod(6), m5)
    m4, m2 = prod(3), prod(1)
    emit(1, 0, _add(m2, m4))
    u = _sub(m3, m2)
    m1 = prod(0)
    emit(0, 0, _add(_add(m1, t), m4))
    emit(1, 1, _add(_add(prod(5), m1), u))


def _strassen2(prod, emit, inner, outer, extra=None):
    done = []

    def outer_prod(R):
        add = extra(R) if extra and done else None
        out = [None] * 4

        def put(i, j, v):
            out[2 * i + j] = v[0] + add[2 * i + j] if add else v[0]

        inner(R)(lambda r: [prod(R, r)], put)
        done.append(R)
        return _add(extra(R), out) if extra and not add else out

    def outer_emit(I, J, tiles):
        for i, j in ((0, 1), (1, 0), (0, 0), (1, 1)):
            emit(2 * I + i, 2 * J + j, tiles[2 * i + j])

    outer(outer_prod, outer_emit)


def _dot(a, b, dims=((1,), (0,))):
    return lax.dot_general(a, b, (dims, ((), ())), preferred_element_type=f32)


def _phi(t):
    return jnp.where(t > 0, t + 1.0, jnp.exp(t)) + 1e-6


def _silu_of_twice(t):
    return t * jnp.tanh(t) + t


def _tile(i):
    return slice(i * T, (i + 1) * T)


def _repeat(v, rows):
    return jnp.concatenate([v] * (rows // 8), axis=0)


def _fold(v):
    acc = v[:8]
    for r in range(8, v.shape[0], 8):
        acc = acc + v[r:r + 8]
    return acc


def _swap_halves(a, b):
    low = lax.broadcasted_iota(i32, a.shape, 1) < T // 2
    moved = pltpu.roll(jnp.where(low, b, a), T // 2, 1)
    return jnp.where(low, a, moved), jnp.where(low, moved, b)


def _store_heads(ref, n, j, v):
    for h in range(T // DH):
        ref[n, pl.ds((j * (T // DH) + h) * PAD, DH), :] = v[h * DH:(h + 1) * DH]


def _load_d_major(ref, n, j):
    return jnp.concatenate(
        [ref[n, pl.ds(4 * j + d, H, stride=PAD), :] for d in range(4)], axis=0)


def _kernel(x_hbm, wqkv_hbm, wo_hbm, wg_hbm, wu_hbm, wd_hbm, gw_hbm, o_hbm,
            x, wk, wu0, w1, w2, gw, out,
            x_sums, wk_sums, pk, hidden, pq, rest, ffn_gate, q_scale,
            z, z_rows, gram_t, gram, m_rows, wq_rows, w_rest, parked,
            zeros, first_sems, sems):
    copy = pltpu.make_async_copy

    def copy_wk(c):
        rows = pl.ds(pl.multiple_of(c * WK_ROWS, WK_ROWS), WK_ROWS)
        return copy(wqkv_hbm.at[:, rows, pl.ds(D, D)], wk.at[:, rows], first_sems.at[c])

    def copy_x(c):
        rows = pl.ds(pl.multiple_of(c * X_ROWS, X_ROWS), X_ROWS)
        return copy(x_hbm.at[:, rows], x.at[:, rows], first_sems.at[T // WK_ROWS + c])

    for c in range(T // WK_ROWS):
        copy_wk(c).start()
    for c in range(Q // X_ROWS):
        copy_x(c).start()

    @pl.loop(0, N_ZEROS // 8)
    def _(n):
        for e in range(8):
            zeros[n * 8 + e] = 0

    used = []

    def zero():
        used.append(None)
        return zeros[len(used) - 1]

    def zero_per_product():
        return functools.lru_cache(None)(lambda R: zero())

    issued = [0]

    def by_mxu(R):
        first = issued[0] % 4
        issued[0] += 7
        if first == 1 and R not in (3, 4):
            return _combine_3_4
        return _combine_4_3 if first < 2 else _combine_spread

    def with_side_jobs(lhs, rhs, dot, jobs):
        tie = zero()
        start = {n * (49 - SIDE_LAG) // len(jobs): job for n, job in enumerate(jobs)}
        assert len(start) == len(jobs)
        due, count = {}, [0]

        def prod(R, r):
            n, b = count[0], rhs(R, r)
            if due.get(n) is not None:
                nothing = pltpu.bitcast(pltpu.bitcast(due[n], i32) & tie, f32)
                b = jnp.concatenate([b[:8] + nothing, b[8:]], axis=0)
            v = dot(lhs(R, r, tie), b.astype(bf16))
            if n in start:
                row = (n % 4) * (v.shape[0] // 8)
                due[n + SIDE_LAG] = start[n](pltpu.bitcast(v[row:row + 8], i32) & tie)
            count[0] += 1
            return v

        return prod, tie

    def project(load, emit, jobs=(), dot=_dot, busy=True):
        prod, tie = with_side_jobs(
            lambda R, r, tie: x_sums[7 * R + r + tie], _operands(_rhs_sum, load), dot, jobs)

        def park(n, tiles):
            for e, v in enumerate(tiles):
                parked[4 * n + e][0] = v
            return lambda: [parked[4 * n + e][tie] for e in range(4)]

        outer = functools.partial(_combine_spread, park=park) if busy else _combine_spread
        _strassen2(prod, lambda i, j, v: emit(i, j, v, tie), by_mxu, outer)

    def tiles_of(ref, n, scale=None):
        off = zero_per_product()

        def load(i, j, R):
            v = ref[n + i + off(R), :, _tile(j)].astype(f32)
            return v if scale is None else v * scale

        return load

    @pl.loop(0, T // WK_ROWS)
    def _(c):
        copy_wk(c).wait()
        rows = pl.ds(pl.multiple_of(c * WK_ROWS, WK_ROWS), WK_ROWS)
        packed_rows = pl.ds(pl.multiple_of(c * (WK_ROWS // 2), WK_ROWS // 2), WK_ROWS // 2)
        w = [[wk[i, rows, _tile(j)].astype(f32) for j in range(4)] for i in range(4)]
        sums = _operands(_rhs_sum, lambda i, j, R: w[i][j])
        for n in range(49):
            wk_sums[n, packed_rows, :] = pltpu.bitcast(sums(n // 7, n % 7).astype(bf16), i32)

    def columns(hbm, start, buf, n, sem):
        return copy(hbm.at[:, :, pl.ds(start, D)], buf.at[pl.ds(n, 4)], sem)

    copy_gw, copy_wu0 = copy(gw_hbm, gw, sems.at[0]), columns(wu_hbm, 0, wu0, 0, sems.at[1])
    sem1, sem2, out_sem = sems.at[2], sems.at[3], sems.at[4]
    copy_gw.start()
    copy_wu0.start()
    for c in (
        columns(wg_hbm, 0, w1, W1_GATE, sem1),
        columns(wu_hbm, D, w1, W1_UP, sem1),
        columns(wg_hbm, D, w1, W1_GATE + 4, sem1),
        columns(wqkv_hbm, 0, w1, W1_Q, sem1),
        copy(wg_hbm.at[:, :, pl.ds(GROUPS * D, REST)],
             w1.at[pl.ds(W1_REST, 4), :, pl.ds(0, REST)], sem1),
        copy(wu_hbm.at[:, :, pl.ds(GROUPS * D, REST)],
             w1.at[pl.ds(W1_REST, 4), :, pl.ds(REST, REST)], sem1),
        columns(wg_hbm, 2 * D, w2, W2_GATE, sem2),
        columns(wu_hbm, 2 * D, w2, W2_UP, sem2),
        columns(wqkv_hbm, 2 * D, w2, W2_V, sem2),
        copy(wo_hbm, w2.at[pl.ds(W2_O, 4)], sem2),
        copy(wd_hbm, w2.at[pl.ds(W2_DOWN, F // T)], sem2),
    ):
        c.start(priority=1)

    z[:4] = jnp.zeros((4, 8, T), f32)

    @pl.loop(0, Q // X_ROWS // X_UNROLL)
    def _(part):
        for c in range(X_UNROLL):
            copy_x(part * X_UNROLL + c).wait()
            rows = pl.ds(pl.multiple_of((part * X_UNROLL + c) * X_ROWS, X_ROWS), X_ROWS)
            sums = _operands(_lhs_sum, lambda i, j, R: x[i, rows, _tile(j)].astype(f32))
            tie = zero()

            def prod(R, r):
                a = sums(R, r)
                x_sums[pl.ds(7 * R + r, 1), rows, :] = a[None].astype(bf16)
                return _dot(a.astype(bf16), pltpu.bitcast(wk_sums[7 * R + r + tie], bf16))

            def emit(i, j, v):
                pk[j, i, rows] = p = _phi(v)
                z[j] += _fold(p)

            _strassen2(prod, emit, lambda R: _combine_spread, _combine_spread)

    copy_gw.wait()
    copy_wu0.wait()

    half_gw = jnp.broadcast_to(gw[...].astype(f32).reshape(1, D) * 0.5, (8, D))

    def mix_gate(i, rows, nothing):
        nothing = pltpu.bitcast(nothing, f32)
        t = [x[i, rows, _tile(j)].astype(f32) * _repeat(half_gw[:, _tile(j)] + nothing, SIDE_ROWS)
             for j in range(4)]
        t = jnp.sum((t[0] + t[1]) + (t[2] + t[3]), axis=1, keepdims=True)
        t = jnp.broadcast_to(0.5 * jnp.tanh(t), (SIDE_ROWS, T))
        ffn_gate[i, rows] = 0.5 - t
        return _fold(t)

    def z_to_rows(j, nothing):
        total = jnp.sum(z[j] + pltpu.bitcast(nothing, f32), axis=0, keepdims=True)
        _store_heads(z_rows, 0, j, jnp.broadcast_to(total, (T, T)).T)

    def z_from_rows(j, nothing):
        v = _load_d_major(z_rows, 0, j) + _repeat(pltpu.bitcast(nothing, f32), T)
        z[4 + j] = v.T[:8]

    def wq_to_rows(i, j, nothing):
        w = pltpu.bitcast(w1[W1_Q + i, :, _tile(j)], i32) | _repeat(nothing, T // 2)
        _store_heads(wq_rows, i, j, pltpu.bitcast(w, bf16).T.astype(f32))

    def pair_rest(i, j, nothing):
        half = _repeat(0.5 + pltpu.bitcast(nothing, f32), T)
        a, b = _swap_halves(w1[W1_REST + i, :, _tile(j)].astype(f32) * half,
                            w1[W1_REST + i, :, _tile(2 + j)].astype(f32))
        w_rest[2 * j, _tile(i)] = a.astype(bf16)
        w_rest[2 * j + 1, _tile(i)] = b.astype(bf16)

    def flip_gram(i, j, nothing):
        g = pltpu.bitcast(gram_t[i, _tile(j)], i32) | _repeat(nothing, T // 2)
        gram[i, :, _tile(j)] = pltpu.bitcast(pltpu.bitcast(g, bf16).T, i32)

    norm_off = zero_per_product()

    def normalise(i, rows, nothing):
        den, off = _repeat(pltpu.bitcast(nothing, f32), SIDE_ROWS), norm_off(0)
        for j in range(4):
            den = den + pq[j + off, i, rows]
        den = den + pltpu.roll(den, 2 * H, 1)
        den = den + pltpu.roll(den, H, 1)
        inverse = pltpu.reciprocal(den + 1e-6, full_range=False)
        q_scale[i, rows] = (1.0 - ffn_gate[i + off, rows]) * inverse

    def over_rows(job):
        return [functools.partial(job, i, pl.ds(r0, SIDE_ROWS))
                for i in range(4) for r0 in range(0, Q, SIDE_ROWS)]

    def over_tiles(job, n):
        return [functools.partial(job, i, j) for i in range(4) for j in range(n)]

    off = zero_per_product()
    over_z = [1.0 / jnp.sum(z[j], axis=0, keepdims=True) for j in range(4)]
    pk_sums = _operands(_lhs_sum, lambda i, j, R: pk[i + off(R), j] * over_z[i])

    def emit_gram(i, j, v):
        gram_t[i, _tile(j)] = v.astype(bf16)

    prod, _ = with_side_jobs(
        lambda R, r, tie: x_sums[7 * RHS_AS_LHS[R] + RHS_AS_LHS[r] + tie], pk_sums,
        functools.partial(_dot, dims=((0,), (0,))), over_rows(mix_gate))
    _strassen2(prod, emit_gram, lambda R: _combine_chain, _combine_chain)

    def up(s, ref, n, jobs=()):
        def emit(i, j, v, tie):
            hidden[s][j, i] = v * ffn_gate[i + tie]

        project(tiles_of(ref, n), emit, jobs, busy=False)

    def gate(s, ref, n, jobs=()):
        def emit(i, j, v, tie):
            u = hidden[s][j + tie, i]
            hidden[s][j + tie, i] = _silu_of_twice(v) * u

        project(tiles_of(ref, n, 0.5), emit, jobs)

    up(0, wu0, 0, [functools.partial(job, j) for job in (z_to_rows, z_from_rows) for j in range(4)])
    copy(w1, w1, sem1).wait()
    gate(0, w1, W1_GATE, over_tiles(pair_rest, 2))
    up(1, w1, W1_UP, over_tiles(wq_to_rows, 4))
    gate(1, w1, W1_GATE + 4, over_tiles(flip_gram, 4))
    pl.delay(1)
    copy(w2, w2, sem2).wait()

    tie = zero()
    same_head = (lax.broadcasted_iota(i32, (T, T), 0) // DH
                 == lax.broadcasted_iota(i32, (T, T), 1) // DH)
    kv = []
    for j in range(4):
        wv = jnp.concatenate([w2[W2_V + i, :, _tile(j)] for i in range(4)], axis=0)
        g = pltpu.bitcast(gram[j + tie], bf16)
        kv.append(jnp.where(same_head, _dot(g, wv), 0.0).astype(bf16))
    for j in range(4):
        m = _dot(kv[j], w2[W2_O + j])
        for n in range(4):
            _store_heads(m_rows, n, j, m[:, _tile(n)])

    def emit_q(i, j, v, tie):
        pq[j, i] = _phi(v) * _repeat(z[4 + j + tie], Q)

    q_off = zero_per_product()
    project(lambda i, j, R: _load_d_major(wq_rows, i + q_off(R), j), emit_q,
            dot=functools.partial(_dot, dims=((1,), (1,))))
    up(2, w2, W2_UP, over_rows(normalise))
    gate(2, w2, W2_GATE)

    waiting = {}

    def emit_rest(i, j, v, tie):
        waiting[i, j] = v
        if (i, j ^ 1) in waiting:
            g, u = _swap_halves(waiting[i, j & 2], waiting[i, j | 1])
            rest[j // 2, i] = _silu_of_twice(g) * (u * ffn_gate[i + tie])

    rest_off = zero_per_product()
    project(lambda i, j, R: w_rest[j + rest_off(R), _tile(i)].astype(f32), emit_rest)

    o = zero_per_product()
    lhs = [_operands(_lhs_sum, lambda i, j, R, s=s: hidden[s][j + o(R), i]) for s in range(GROUPS)]
    lhs.append(_operands(_lhs_sum, lambda i, j, R: pq[j + o(R), i] * q_scale[i + o(R)]))
    rhs = [_operands(_rhs_sum,
                     lambda i, j, R, s=s: w2[W2_DOWN + 4 * s + i + o(R), :, _tile(j)].astype(f32))
           for s in range(GROUPS)]
    rhs.append(_operands(_rhs_sum, lambda i, j, R: _load_d_major(m_rows, j + o(R), i)))

    def prod_out(R, r):
        return _dot(jnp.concatenate([a(R, r) for a in lhs], axis=1).astype(bf16),
                    jnp.concatenate([b(R, r) for b in rhs], axis=0).astype(bf16))

    def prod_rest(R):
        a = _lhs_sum(R, lambda I, J: [rest[J + o(R), 2 * I + i] for i in range(2)])
        b = _rhs_sum(R, lambda I, J: [
            w2[W2_DOWN + 4 * GROUPS + I + o(R), :, _tile(2 * J + j)].astype(f32) for j in range(2)])
        return [_dot(a[i].astype(bf16), b[j].astype(bf16)) for i in range(2) for j in range(2)]

    written = []

    def emit_out(i, j, v):
        written.append(None)
        cuts = (0, Q) if len(written) < 16 else (0, 3 * Q // 4, Q)
        for lo, hi in zip(cuts, cuts[1:]):
            out[j, i, lo:hi] = v[lo:hi].astype(bf16)
            copy(out.at[j, i, lo:hi], o_hbm.at[i, lo:hi, _tile(j)], out_sem).start()

    _strassen2(prod_out, emit_out, lambda R: _combine_chain, _combine_chain, prod_rest)
    copy(o_hbm, o_hbm, out_sem).wait()


@jax.jit
def pallas_gated_mix__linear_attn_block__swiglu_ffn__prompt_kernel(
    A_x: jax.Array,
    A_wqkv: jax.Array,
    A_wo: jax.Array,
    B_x: jax.Array,
    B_w_gate: jax.Array,
    B_w_up: jax.Array,
    B_w_down: jax.Array,
    gate_w: jax.Array,
):
    del B_x
    vmem = pltpu.VMEM
    tiles = vmem((4, 4, Q, T), f32)
    out = pl.pallas_call(
        _kernel,
        in_specs=[pl.BlockSpec(memory_space=pl.ANY)] * 7,
        out_specs=pl.BlockSpec(memory_space=pl.ANY),
        out_shape=jax.ShapeDtypeStruct((4, Q, D), bf16),
        scratch_shapes=[
            vmem((4, Q, D), bf16),
            vmem((4, T, D), bf16),
            vmem((4, T, D), bf16),
            vmem((W1_SIZE, T, D), bf16),
            vmem((W2_SIZE, T, D), bf16),
            vmem((D,), bf16),
            vmem((4, 4, Q, T), bf16),
            vmem((49, Q, T), bf16),
            vmem((49, T // 2, T), i32),
            tiles,
            [tiles] * GROUPS,
            tiles,
            vmem((2, 4, Q, T), f32),
            vmem((4, Q, T), f32),
            vmem((4, Q, T), f32),
            vmem((8, 8, T), f32),
            vmem((1, PAD_ROWS, T), f32),
            vmem((4, D, T), bf16),
            vmem((4, T // 2, D), i32),
            vmem((4, PAD_ROWS, T), f32),
            vmem((4, PAD_ROWS, T), f32),
            vmem((4, D, T), bf16),
            [vmem((2, Q, T), f32)] * 8,
            pltpu.SMEM((N_ZEROS,), i32),
            pltpu.SemaphoreType.DMA((T // WK_ROWS + Q // X_ROWS,)),
            pltpu.SemaphoreType.DMA((5,)),
        ],
        compiler_params=pltpu.CompilerParams(
            vmem_limit_bytes=100 * 1024 * 1024,
            disable_semaphore_checks=True,
            flags={"XLA_TPU_RESCHEDULE_DMA_DONES": True},
        ),
    )(
        A_x.reshape(4, Q, D),
        A_wqkv.reshape(4, T, 3 * D),
        A_wo.reshape(4, T, D),
        B_w_gate.reshape(4, T, F),
        B_w_up.reshape(4, T, F),
        B_w_down.reshape(F // T, T, D),
        gate_w,
    )
    return out.reshape(1, S, D)
```
